```python
import os as _os
_os.environ.setdefault("JAX_PLATFORMS", "cpu")
import jax
import jax.numpy as jnp

def _softmax(x, axis=-1):
    return jax.nn.softmax(x, axis=axis)
def _gelu(x):
    return jax.nn.gelu(x, approximate=True)
def _silu(x):
    return jax.nn.silu(x)
def _sigmoid(x):
    return jax.nn.sigmoid(x)
def _layernorm(x, axis=-1, eps=1e-5):
    m = jnp.mean(x, axis=axis, keepdims=True)
    v = jnp.var(x, axis=axis, keepdims=True)
    return (x - m) / jnp.sqrt(v + eps)
def _scatter_add(tgt, idx, src, axis=0):
    return tgt.at[idx].add(src)
def _segment_sum(src, seg, n):
    return jax.ops.segment_sum(src, seg, n)
class _Rng:
    def __init__(self, key):
        self._k = key
    def _next(self):
        self._k, sub = jax.random.split(self._k)
        return sub
    def normal(self, shape):
        return jax.random.normal(self._next(), shape, dtype=jnp.bfloat16)
    def randint(self, lo, hi, shape):
        return jax.random.randint(self._next(), shape, lo, hi, dtype=jnp.int32)
    def uniform(self, shape, lo=0.0, hi=1.0):
        return jax.random.uniform(self._next(), shape, jnp.bfloat16, lo, hi)
    def permutation(self, n):
        return jax.random.permutation(self._next(), n)


kernel_name = 'gated_mix__mha_block__softmax_full_mha__prompt'

def setup_inputs():
    _rng = _Rng(jax.random.key(int.from_bytes(__import__("os").urandom(4), "little")))
    _w = (lambda a: (lambda t: t.astype(jnp.bfloat16) if jnp.issubdtype(t.dtype, jnp.floating) else t)(jnp.asarray(a)))
    def _A_setup():
        B, S, D, H = 1, 2048, 448, 16
        return {
            "x": _w((lambda *s: _rng.normal(s) * 0.05)(B, S, D)),
            "wqkv": _w((lambda *s: _rng.normal(s) * 0.4)(D, 3 * D)),
            "wo": _w((lambda *s: _rng.normal(s) * 0.05)(D, D)),
        }
    _A_in = _A_setup()

    def _B_setup():
        B, S, D = 1, 2048, 448
        return {
            "x": _w((lambda *s: _rng.normal(s) * 0.05)(B, S, D)),
            "wqkv": _w((lambda *s: _rng.normal(s) * 0.4)(D, 3 * D)),
            "wo": _w((lambda *s: _rng.normal(s) * 0.05)(D, D)),
        }
    _B_in = _B_setup()

    return {
        "A_x": _A_in["x"],
        "A_wqkv": _A_in["wqkv"],
        "A_wo": _A_in["wo"],
        "B_x": _B_in["x"],
        "B_wqkv": _B_in["wqkv"],
        "B_wo": _B_in["wo"],
        "gate_w": _w((lambda *s: _rng.normal(s) * 0.05)(448) * 16.0),
    }

def reference(A_x, A_wqkv, A_wo, B_x, B_wqkv, B_wo, gate_w):
    def _A_ref(x, wqkv, wo):
        B, S, D = x.shape
        H = 16
        Dh = D // H
        qkv = (lambda x, *d: x.transpose(*d))((x @ wqkv).reshape(B, S, 3, H, Dh), 2, 0, 3, 1, 4)
        q, k, v = qkv[0], qkv[1], qkv[2]
        scores = jnp.einsum("bhqd,bhkd->bhqk", q, k) * (Dh ** -0.5)
        p = _softmax(scores, axis=-1)
        o = jnp.einsum("bhqk,bhkd->bhqd", p, v)
        return (lambda x, *d: x.transpose(*d))(o, 0, 2, 1, 3).reshape(B, S, D) @ wo

    def _B_ref(x, wqkv, wo):
        B, S, D = x.shape
        H = 16; Dh = D // H
        qkv = (lambda x, *d: x.transpose(*d))((x @ wqkv).reshape(B, S, 3, H, Dh), 2, 0, 3, 1, 4)
        q, k, v = qkv[0], qkv[1], qkv[2]
        scale = Dh ** -0.5
        scores = jnp.einsum("bhqd,bhkd->bhqk", q, k) * scale
        p = _softmax(scores, axis=-1)
        o = jnp.einsum("bhqk,bhkd->bhqd", p, v)
        return (lambda x, *d: x.transpose(*d))(o, 0, 2, 1, 3).reshape(B, S, D) @ wo

    x = A_x
    g = _sigmoid((x * gate_w).sum(-1, keepdims=True))
    a = _A_ref(x, A_wqkv, A_wo)
    b = _B_ref(x, B_wqkv, B_wo)
    return g * a + (1 - g) * b
```

```python
import math

import jax
import jax.numpy as jnp
import jax.experimental.pallas as pl
import jax.experimental.pallas.tpu as pltpu

S = 2048
D = 448
H = 16
DH = 28
HP = 32
DP = H * HP
NG = DP // 128
TQ = 256
NQ = S // TQ
_C = (DH ** -0.5) * math.log2(math.e)

_NT = (((1,), (1,)), ((), ()))


def _kernel(x_ref, wqt_ref, wvt_ref, wk_ref, wot_ref, gate_ref, out_ref,
            qt_s, k_s, vt_s, gl_s, ot_s):
    step = pl.program_id(0)

    @pl.when(step == 0)
    def _():
        x = x_ref[...]
        for br in range(2):
            qt = jax.lax.dot_general(wqt_ref[br], x, _NT,
                                     preferred_element_type=jnp.float32) * _C
            qt = qt.astype(jnp.bfloat16)
            for g in range(NG):
                qt_s[br * NG + g] = qt[g * 128:(g + 1) * 128, :]
            vt = jax.lax.dot_general(wvt_ref[br], x, _NT,
                                     preferred_element_type=jnp.float32)
            row = jax.lax.broadcasted_iota(jnp.int32, (DP, S), 0)
            vt = jnp.where((row % HP) == DH, 1.0, vt).astype(jnp.bfloat16)
            for h in range(H):
                vt_s[br * H + h] = vt[h * HP:(h + 1) * HP, :]
            k = jnp.dot(x, wk_ref[br], preferred_element_type=jnp.float32)
            k = k.astype(jnp.bfloat16)
            for g in range(NG):
                k_s[br * NG + g] = k[:, g * 128:(g + 1) * 128]
        gl_s[...] = jax.lax.dot_general(gate_ref[...], x, _NT,
                                        preferred_element_type=jnp.float32)

    q0 = pl.multiple_of(step * TQ, TQ)
    rowg = jax.lax.broadcasted_iota(jnp.int32, (128, TQ), 0) // HP

    def unit(u):
        g = u // 4
        sub = u % 4
        qg = qt_s[g, :, pl.ds(q0, TQ)]
        qm = jnp.where(rowg == sub, qg, jnp.zeros_like(qg))
        s = jnp.dot(k_s[g], qm, preferred_element_type=jnp.float32)
        m = jnp.max(s, axis=0, keepdims=True)
        p = jnp.exp2(s - m).astype(jnp.bfloat16)
        o = jnp.dot(vt_s[u], p, preferred_element_type=jnp.float32)
        o = o * (1.0 / o[DH:DH + 1, :])
        ot_s[u] = o.astype(jnp.bfloat16)

    def body(i, carry):
        unit(i)
        unit(i + H)
        return carry

    jax.lax.fori_loop(0, H, body, 0)

    ot = ot_s[...].reshape(2 * DP, TQ)
    at = jnp.dot(wot_ref[0], ot[:DP], preferred_element_type=jnp.float32)
    bt = jnp.dot(wot_ref[1], ot[DP:], preferred_element_type=jnp.float32)
    gl = gl_s[0:1, pl.ds(q0, TQ)]
    gt = jax.nn.sigmoid(gl)
    res = gt * at + (1.0 - gt) * bt
    out_ref[...] = res.T[:, :D].astype(out_ref.dtype)


def _pad_heads_cols(w):
    return jnp.pad(w.reshape(D, H, DH), ((0, 0), (0, 0), (0, HP - DH))).reshape(D, DP)


@jax.jit
def pallas_gated_mix__mha_block__softmax_full_mha__prompt_kernel(
    A_x: jax.Array,
    A_wqkv: jax.Array,
    A_wo: jax.Array,
    B_x: jax.Array,
    B_wqkv: jax.Array,
    B_wo: jax.Array,
    gate_w: jax.Array,
):
    x = A_x.reshape(S, D)
    wqkv = jnp.stack([A_wqkv, B_wqkv])
    wqkv = jnp.pad(wqkv.reshape(2, D, 3 * H, DH),
                   ((0, 0), (0, 0), (0, 0), (0, HP - DH))).reshape(2, D, 3, DP)
    wqt = wqkv[:, :, 0, :].transpose(0, 2, 1)
    wk = wqkv[:, :, 1, :]
    wvt = wqkv[:, :, 2, :].transpose(0, 2, 1)
    wo = jnp.stack([A_wo, B_wo])
    wo = jnp.pad(wo.reshape(2, H, DH, D),
                 ((0, 0), (0, 0), (0, HP - DH), (0, DP - D))).reshape(2, DP, DP)
    wot = wo.transpose(0, 2, 1)
    gate8 = jnp.pad(gate_w.reshape(1, D), ((0, 7), (0, 0)))

    out = pl.pallas_call(
        _kernel,
        grid=(NQ,),
        in_specs=[
            pl.BlockSpec((S, D), lambda i: (0, 0)),
            pl.BlockSpec((2, DP, D), lambda i: (0, 0, 0)),
            pl.BlockSpec((2, DP, D), lambda i: (0, 0, 0)),
            pl.BlockSpec((2, D, DP), lambda i: (0, 0, 0)),
            pl.BlockSpec((2, DP, DP), lambda i: (0, 0, 0)),
            pl.BlockSpec((8, D), lambda i: (0, 0)),
        ],
        out_specs=pl.BlockSpec((TQ, D), lambda i: (i, 0)),
        out_shape=jax.ShapeDtypeStruct((S, D), jnp.bfloat16),
        scratch_shapes=[
            pltpu.VMEM((2 * NG, 128, S), jnp.bfloat16),
            pltpu.VMEM((2 * NG, S, 128), jnp.bfloat16),
            pltpu.VMEM((2 * H, HP, S), jnp.bfloat16),
            pltpu.VMEM((8, S), jnp.float32),
            pltpu.VMEM((2 * H, HP, TQ), jnp.bfloat16),
        ],
        compiler_params=pltpu.CompilerParams(
            dimension_semantics=("arbitrary",),
            vmem_limit_bytes=100 * 1024 * 1024,
        ),
    )(x, wqt, wvt, wk, wot, gate8)
    return out.reshape(1, S, D)
```

```python
import math, os

import jax
import jax.numpy as jnp
import jax.experimental.pallas as pl
import jax.experimental.pallas.tpu as pltpu

S = 2048
D = 448
H = 16
DH = 28
HP = 32
DP = H * HP
NG = DP // 128
TQ = 512
NQ = S // TQ
KC = 256
NC = S // KC
_C = (DH ** -0.5) * math.log2(math.e)

_TN = (((0,), (0,)), ((), ()))


def _kernel(xt_ref, wa_ref, wb_ref, woa_ref, wob_ref, gate_ref, out_ref,
            qt_s, k_s, vt_s, gl_s, ot_s, wot_s, sa_s, sb_s, ma_s, mb_s):
    step = pl.program_id(0)
    rowg = jax.lax.broadcasted_iota(jnp.int32, (128, TQ), 0) // HP

    def load_qm(u, q0):
        qg = qt_s[u // 4, :, pl.ds(q0, TQ)]
        return jnp.where(rowg == (u % 4), qg, jnp.zeros_like(qg))

    def phase(u_cur, s_cur, m_cur_ref, u_nxt, q_nxt, s_nxt, m_nxt_ref):
        qm = load_qm(u_nxt, q_nxt)
        gn = u_nxt // 4
        mrun = None
        acc = None
        if u_cur is not None:
            m_cur = m_cur_ref[...]
        for c in range(NC):
            rows = slice(c * KC, (c + 1) * KC)
            sn = jnp.dot(k_s[gn, rows, :], qm, preferred_element_type=jnp.float32)
            s_nxt[rows, :] = sn
            mc = jnp.max(sn.reshape(KC // 8, 8, TQ), axis=0)
            mrun = mc if mrun is None else jnp.maximum(mrun, mc)
            if u_cur is not None:
                p = jnp.exp2(s_cur[rows, :] - m_cur).astype(jnp.bfloat16)
                o = jnp.dot(vt_s[u_cur, :, rows], p, preferred_element_type=jnp.float32)
                acc = o if acc is None else acc + o
        m_nxt_ref[...] = jnp.max(mrun, axis=0, keepdims=True)
        if u_cur is not None:
            acc = acc * (1.0 / acc[DH:DH + 1, :])
            ot_s[u_cur] = acc.astype(jnp.bfloat16)

    @pl.when(step == 0)
    def _():
        xt = xt_ref[...]
        row4 = jax.lax.broadcasted_iota(jnp.int32, (HP - DH, S), 0)
        zpad = jnp.zeros((HP - DH, S), jnp.float32)
        onepad = jnp.where(row4 == 0, 1.0, 0.0)
        for br, (w_ref, wo_ref) in enumerate(((wa_ref, woa_ref), (wb_ref, wob_ref))):
            qkv = jax.lax.dot_general(w_ref[...], xt, _TN,
                                      preferred_element_type=jnp.float32)
            def head(t, h, pad):
                r0 = t * D + h * DH
                return jnp.concatenate([qkv[r0:r0 + DH, :], pad], axis=0)
            for g in range(NG):
                qg = jnp.concatenate([head(0, 4 * g + i, zpad) for i in range(4)], axis=0)
                qt_s[br * NG + g] = (qg * _C).astype(jnp.bfloat16)
                kg = jnp.concatenate([head(1, 4 * g + i, zpad) for i in range(4)], axis=0)
                k_s[br * NG + g] = kg.T.astype(jnp.bfloat16)
            for h in range(H):
                vt_s[br * H + h] = head(2, h, onepad).astype(jnp.bfloat16)
            wo = wo_ref[...].astype(jnp.float32)
            zw = jnp.zeros((HP - DH, D), jnp.float32)
            wop = jnp.concatenate(
                [jnp.concatenate([wo[h * DH:(h + 1) * DH, :], zw], axis=0) for h in range(H)],
                axis=0)
            wot_s[br] = wop.T.astype(jnp.bfloat16)
        gl_s[...] = jnp.dot(gate_ref[...], xt, preferred_element_type=jnp.float32)
        phase(None, None, None, 0, 0, sa_s, ma_s)

    q0 = pl.multiple_of(step * TQ, TQ)
    q_next_tile = pl.multiple_of(jnp.minimum(step + 1, NQ - 1) * TQ, TQ)

    def body(j, carry):
        u0 = 2 * j
        phase(u0, sa_s, ma_s, u0 + 1, q0, sb_s, mb_s)
        un = u0 + 2
        wrap = un >= 2 * H
        un = jnp.where(wrap, 0, un)
        qn = pl.multiple_of(jnp.where(wrap, q_next_tile, q0), TQ)
        phase(u0 + 1, sb_s, mb_s, un, qn, sa_s, ma_s)
        return carry

    jax.lax.fori_loop(0, H, body, 0)

    ot = ot_s[...].reshape(2 * DP, TQ)
    at = jnp.dot(wot_s[0], ot[:DP], preferred_element_type=jnp.float32)
    bt = jnp.dot(wot_s[1], ot[DP:], preferred_element_type=jnp.float32)
    gl = gl_s[0:1, pl.ds(q0, TQ)]
    gt = jax.nn.sigmoid(gl)
    res = gt * at + (1.0 - gt) * bt
    out_ref[...] = res.astype(out_ref.dtype)


@jax.jit
def pallas_gated_mix__mha_block__softmax_full_mha__prompt_kernel(
    A_x: jax.Array,
    A_wqkv: jax.Array,
    A_wo: jax.Array,
    B_x: jax.Array,
    B_wqkv: jax.Array,
    B_wo: jax.Array,
    gate_w: jax.Array,
):
    xt = A_x.reshape(S, D).T
    gate8 = jnp.pad(gate_w.reshape(1, D), ((0, 7), (0, 0)))

    out = pl.pallas_call(
        _kernel,
        grid=(NQ,),
        in_specs=[
            pl.BlockSpec((D, S), lambda i: (0, 0)),
            pl.BlockSpec((D, 3 * D), lambda i: (0, 0)),
            pl.BlockSpec((D, 3 * D), lambda i: (0, 0)),
            pl.BlockSpec((D, D), lambda i: (0, 0)),
            pl.BlockSpec((D, D), lambda i: (0, 0)),
            pl.BlockSpec((8, D), lambda i: (0, 0)),
        ],
        out_specs=pl.BlockSpec((D, TQ), lambda i: (0, i)),
        out_shape=jax.ShapeDtypeStruct((D, S), jnp.bfloat16),
        scratch_shapes=[
            pltpu.VMEM((2 * NG, 128, S), jnp.bfloat16),
            pltpu.VMEM((2 * NG, S, 128), jnp.bfloat16),
            pltpu.VMEM((2 * H, HP, S), jnp.bfloat16),
            pltpu.VMEM((8, S), jnp.float32),
            pltpu.VMEM((2 * H, HP, TQ), jnp.bfloat16),
            pltpu.VMEM((2, D, DP), jnp.bfloat16),
            pltpu.VMEM((S, TQ), jnp.float32),
            pltpu.VMEM((S, TQ), jnp.float32),
            pltpu.VMEM((1, TQ), jnp.float32),
            pltpu.VMEM((1, TQ), jnp.float32),
        ],
        compiler_params=pltpu.CompilerParams(
            dimension_semantics=("arbitrary",),
            vmem_limit_bytes=100 * 1024 * 1024,
        ),
    )(xt, A_wqkv, B_wqkv, A_wo, B_wo, gate8)
    return out.T.reshape(1, S, D)
```

```python
import math

import jax
import jax.numpy as jnp
import jax.experimental.pallas as pl
import jax.experimental.pallas.tpu as pltpu

S = 2048
D = 448
H = 16
DH = 28
HP = 32
DP = H * HP
NG = DP // 128
TQ = 512
NQ = S // TQ
KC = 128
NC = S // KC
UN = 8
LAG = 2
XC = 512
NX = S // XC
_C = (DH ** -0.5) * math.log2(math.e)


def _kernel(xt_hbm, wa_hbm, wb_hbm, woa_hbm, wob_hbm, gate_ref, out_ref,
            xt_s, w_s, wo_s, sems,
            qt_s, k_s, vt_s, gl_s, ot_s, wot_s, sa_s, sb_s, ma_s, mb_s):
    step = pl.program_id(0)
    rowg = jax.lax.broadcasted_iota(jnp.int32, (128, TQ), 0) // HP

    def load_qm(u, q0):
        qg = qt_s[u // 4, :, pl.ds(q0, TQ)]
        return jnp.where(rowg == (u % 4), qg, jnp.zeros_like(qg))

    def phase(u_cur, s_cur, m_cur_ref, u_nxt, q_nxt, s_nxt, m_nxt_ref):
        qm = load_qm(u_nxt, q_nxt)
        gn = u_nxt // 4
        st = dict(mrun=None, acc=None)
        if u_cur is not None:
            m_cur = m_cur_ref[...]

        def qk(c):
            rows = slice(c * KC, (c + 1) * KC)
            sn = jnp.dot(k_s[gn, rows, :], qm, preferred_element_type=jnp.float32)
            s_nxt[rows, :] = sn
            mc = jnp.max(sn.reshape(KC // 8, 8, TQ), axis=0)
            st["mrun"] = mc if st["mrun"] is None else jnp.maximum(st["mrun"], mc)

        def pv(c):
            if u_cur is None:
                return
            rows = slice(c * KC, (c + 1) * KC)
            p = jnp.exp2(s_cur[rows, :] - m_cur).astype(jnp.bfloat16)
            o = jnp.dot(vt_s[u_cur, :, rows], p, preferred_element_type=jnp.float32)
            st["acc"] = o if st["acc"] is None else st["acc"] + o

        for c in range(NC + LAG):
            if c < NC:
                qk(c)
            if c >= LAG:
                pv(c - LAG)
        m_nxt_ref[...] = jnp.max(st["mrun"], axis=0, keepdims=True)
        if u_cur is not None:
            acc = st["acc"]
            acc = acc * (1.0 / acc[DH:DH + 1, :])
            ot_s[u_cur] = acc.astype(jnp.bfloat16)

    @pl.when(step == 0)
    def _():
        cp_w = [pltpu.make_async_copy(wa_hbm, w_s.at[0], sems.at[0]),
                pltpu.make_async_copy(wb_hbm, w_s.at[1], sems.at[1])]
        cp_wo = [pltpu.make_async_copy(woa_hbm, wo_s.at[0], sems.at[2]),
                 pltpu.make_async_copy(wob_hbm, wo_s.at[1], sems.at[3])]
        cp_x = [pltpu.make_async_copy(xt_hbm.at[:, pl.ds(i * XC, XC)],
                                      xt_s.at[:, pl.ds(i * XC, XC)], sems.at[4 + i])
                for i in range(NX)]
        cp_w[0].start()
        for c in cp_x:
            c.start()
        cp_w[1].start()
        cp_wo[0].start()
        cp_wo[1].start()

        row4 = jax.lax.broadcasted_iota(jnp.int32, (HP - DH, XC), 0)
        zpad = jnp.zeros((HP - DH, XC), jnp.float32)
        onepad = jnp.where(row4 == 0, 1.0, 0.0)
        cp_w[0].wait()
        cp_x[0].wait()
        for br in range(2):
            wt = w_s[br].T
            for i in range(NX):
                if br == 0 and i == 1:
                    for c in cp_x[1:]:
                        c.wait()
                    cp_w[1].wait()
                    cp_wo[0].wait()
                    cp_wo[1].wait()
                cols = slice(i * XC, (i + 1) * XC)
                xt = xt_s[:, cols]
                qkv = jnp.dot(wt, xt, preferred_element_type=jnp.float32)

                def head(t, h, pad):
                    r0 = t * D + h * DH
                    return jnp.concatenate([qkv[r0:r0 + DH, :], pad], axis=0)

                for g in range(NG):
                    qg = jnp.concatenate([head(0, 4 * g + j, zpad) for j in range(4)], axis=0)
                    qt_s[br * NG + g, :, cols] = (qg * _C).astype(jnp.bfloat16)
                    kg = jnp.concatenate([head(1, 4 * g + j, zpad) for j in range(4)], axis=0)
                    k_s[br * NG + g, cols, :] = kg.T.astype(jnp.bfloat16)
                for h in range(H):
                    vt_s[br * H + h, :, cols] = head(2, h, onepad).astype(jnp.bfloat16)
                if br == 0:
                    gl_s[:, cols] = jnp.dot(gate_ref[...], xt,
                                            preferred_element_type=jnp.float32)
            wo = wo_s[br].astype(jnp.float32)
            zw = jnp.zeros((HP - DH, D), jnp.float32)
            wop = jnp.concatenate(
                [jnp.concatenate([wo[h * DH:(h + 1) * DH, :], zw], axis=0) for h in range(H)],
                axis=0)
            wot_s[br] = wop.T.astype(jnp.bfloat16)
        phase(None, None, None, 0, 0, sa_s, ma_s)

    q0 = pl.multiple_of(step * TQ, TQ)
    q_next_tile = pl.multiple_of(jnp.minimum(step + 1, NQ - 1) * TQ, TQ)

    def body(j, carry):
        u0 = UN * j
        bufs = [(sa_s, ma_s), (sb_s, mb_s)]
        for r in range(UN):
            cur = bufs[r % 2]
            nxt = bufs[(r + 1) % 2]
            if r < UN - 1:
                phase(u0 + r, cur[0], cur[1], u0 + r + 1, q0, nxt[0], nxt[1])
            else:
                un = u0 + UN
                wrap = un >= 2 * H
                un = jnp.where(wrap, 0, un)
                qn = pl.multiple_of(jnp.where(wrap, q_next_tile, q0), TQ)
                phase(u0 + r, cur[0], cur[1], un, qn, nxt[0], nxt[1])
        return carry

    jax.lax.fori_loop(0, 2 * H // UN, body, 0)

    ot = ot_s[...].reshape(2 * DP, TQ)
    at = jnp.dot(wot_s[0], ot[:DP], preferred_element_type=jnp.float32)
    bt = jnp.dot(wot_s[1], ot[DP:], preferred_element_type=jnp.float32)
    gl = gl_s[0:1, pl.ds(q0, TQ)]
    gt = jax.nn.sigmoid(gl)
    res = gt * at + (1.0 - gt) * bt
    out_ref[...] = res.astype(out_ref.dtype)


@jax.jit
def pallas_gated_mix__mha_block__softmax_full_mha__prompt_kernel(
    A_x: jax.Array,
    A_wqkv: jax.Array,
    A_wo: jax.Array,
    B_x: jax.Array,
    B_wqkv: jax.Array,
    B_wo: jax.Array,
    gate_w: jax.Array,
):
    del B_x
    xt = A_x.reshape(S, D).T
    gate8 = jnp.pad(gate_w.reshape(1, D), ((0, 7), (0, 0)))

    out = pl.pallas_call(
        _kernel,
        grid=(NQ,),
        in_specs=[
            pl.BlockSpec(memory_space=pl.ANY),
            pl.BlockSpec(memory_space=pl.ANY),
            pl.BlockSpec(memory_space=pl.ANY),
            pl.BlockSpec(memory_space=pl.ANY),
            pl.BlockSpec(memory_space=pl.ANY),
            pl.BlockSpec((8, D), lambda i: (0, 0)),
        ],
        out_specs=pl.BlockSpec((D, TQ), lambda i: (0, i)),
        out_shape=jax.ShapeDtypeStruct((D, S), jnp.bfloat16),
        scratch_shapes=[
            pltpu.VMEM((D, S), jnp.bfloat16),
            pltpu.VMEM((2, D, 3 * D), jnp.bfloat16),
            pltpu.VMEM((2, D, D), jnp.bfloat16),
            pltpu.SemaphoreType.DMA((4 + NX,)),
            pltpu.VMEM((2 * NG, 128, S), jnp.bfloat16),
            pltpu.VMEM((2 * NG, S, 128), jnp.bfloat16),
            pltpu.VMEM((2 * H, HP, S), jnp.bfloat16),
            pltpu.VMEM((8, S), jnp.float32),
            pltpu.VMEM((2 * H, HP, TQ), jnp.bfloat16),
            pltpu.VMEM((2, D, DP), jnp.bfloat16),
            pltpu.VMEM((S, TQ), jnp.float32),
            pltpu.VMEM((S, TQ), jnp.float32),
            pltpu.VMEM((1, TQ), jnp.float32),
            pltpu.VMEM((1, TQ), jnp.float32),
        ],
        compiler_params=pltpu.CompilerParams(
            dimension_semantics=("arbitrary",),
            vmem_limit_bytes=100 * 1024 * 1024,
        ),
    )(xt, A_wqkv, B_wqkv, A_wo, B_wo, gate8)
    return out.T.reshape(1, S, D)
```
